```python
import jax
import jax.numpy as jnp

def _softmax(x, axis=-1):
    return jax.nn.softmax(x, axis=axis)
def _gelu(x):
    return jax.nn.gelu(x, approximate=True)
def _silu(x):
    return jax.nn.silu(x)
def _sigmoid(x):
    return jax.nn.sigmoid(x)
def _layernorm(x, axis=-1, eps=1e-5):
    m = jnp.mean(x, axis=axis, keepdims=True)
    v = jnp.var(x, axis=axis, keepdims=True)
    return (x - m) / jnp.sqrt(v + eps)
def _scatter_add(tgt, idx, src, axis=0):
    return tgt.at[idx].add(src)
def _segment_sum(src, seg, n):
    return jax.ops.segment_sum(src, seg, n)
class _Rng:
    def __init__(self, key):
        self._k = key
    def _next(self):
        self._k, sub = jax.random.split(self._k)
        return sub
    def normal(self, shape):
        return jax.random.normal(self._next(), shape, dtype=jnp.bfloat16)
    def randint(self, lo, hi, shape):
        return jax.random.randint(self._next(), shape, lo, hi, dtype=jnp.int32)
    def uniform(self, shape, lo=0.0, hi=1.0):
        return jax.random.uniform(self._next(), shape, jnp.bfloat16, lo, hi)
    def permutation(self, n):
        return jax.random.permutation(self._next(), n)


kernel_name = 'parallel_sum__sliding_block_cached__moe_arch_mod__decode'

def setup_inputs():
    _rng = _Rng(jax.random.key(int.from_bytes(__import__("os").urandom(4), "little")))
    _w = (lambda a: (lambda t: t.astype(jnp.bfloat16) if jnp.issubdtype(t.dtype, jnp.floating) else t)(jnp.asarray(a)))
    def _A_setup():
        B, Sq, D = 1, 1, 512
        Hq, Hkv, Sk, Dh = 32, 8, 65536, 128
        assert Hq % Hkv == 0, (Hq, Hkv)
        return {
            "x": _w((lambda *s: _rng.normal(s) * 0.05)(B, Sq, D)),
            "k_cache": _w((lambda *s: _rng.normal(s) * 0.05)(B, Hkv, Sk, Dh)),
            "v_cache": _w((lambda *s: _rng.normal(s) * 0.05)(B, Hkv, Sk, Dh)),
            "wq": _w((lambda *s: _rng.normal(s) * 0.05)(D, Hq * Dh) * (D ** -0.5)),
            "wo": _w((lambda *s: _rng.normal(s) * 0.05)(Hq * Dh, D) * ((Hq * Dh) ** -0.5)),
        }
    _A_in = _A_setup()

    def _B_setup():
        B, S, D, F, C = 1, 1, 512, 1792, 1
        return {
            "x": _w((lambda *s: _rng.normal(s) * 0.05)(B, S, D)),
            "w_r": _w((lambda *s: _rng.normal(s) * 0.05)(D)),
            "w_gate": _w((lambda *s: _rng.normal(s) * 0.05)(D, F)),
            "w_up": _w((lambda *s: _rng.normal(s) * 0.05)(D, F)),
            "w_down": _w((lambda *s: _rng.normal(s) * 0.05)(F, D)),
        }
    _B_in = _B_setup()

    return {
        "A_x": _A_in["x"],
        "A_k_cache": _A_in["k_cache"],
        "A_v_cache": _A_in["v_cache"],
        "A_wq": _A_in["wq"],
        "A_wo": _A_in["wo"],
        "B_x": _B_in["x"],
        "B_w_r": _B_in["w_r"],
        "B_w_gate": _B_in["w_gate"],
        "B_w_up": _B_in["w_up"],
        "B_w_down": _B_in["w_down"],
    }

def reference(A_x, A_k_cache, A_v_cache, A_wq, A_wo, B_x, B_w_r, B_w_gate, B_w_up, B_w_down):
    def _A_ref(x, k_cache, v_cache, wq, wo):
        B, Sq, D = x.shape
        Hq, Dh = 32, 128
        Hkv, Sk = k_cache.shape[1], k_cache.shape[2]
        W = min(4096, max(256, Sk // 4))
        rep = Hq // Hkv
        q = (lambda x, *d: x.transpose(*d))((x @ wq).reshape(B, Sq, Hq, Dh), 0, 2, 1, 3)
        k = jnp.repeat(k_cache[:, :, Sk - W:, :], rep, axis=1)
        v = jnp.repeat(v_cache[:, :, Sk - W:, :], rep, axis=1)
        scores = jnp.einsum("bhqd,bhkd->bhqk", q, k) * (Dh ** -0.5)
        p = _softmax(scores, axis=-1)
        o = jnp.einsum("bhqk,bhkd->bhqd", p, v)
        return (lambda x, *d: x.transpose(*d))(o, 0, 2, 1, 3).reshape(B, Sq, Hq * Dh) @ wo

    def _B_ref(x, w_r, w_gate, w_up, w_down):
        B, S, D = x.shape
        C = 1
        r = x @ w_r
        idx = jnp.argsort(-r, axis=-1)[:, :C]
        idx_e = jnp.repeat(idx.reshape(B, C, 1), D, axis=2)
        x_sel = jnp.take_along_axis(x, idx_e, axis=1)
        g = _silu(x_sel @ w_gate)
        u = x_sel @ w_up
        y = (g * u) @ w_down
        r_sel = _sigmoid(jnp.take_along_axis(r, idx, axis=1))
        y = y * r_sel.reshape(B, C, 1)
        b_off = (jnp.arange(B) * S).reshape(B, 1)
        flat_idx = (idx + b_off).reshape(B * C)
        zero = (x * 0.0).reshape(B * S, D)
        upd = _scatter_add(zero, flat_idx, y.reshape(B * C, D), axis=0)
        return x + upd.reshape(B, S, D)

    x = A_x
    xn = _layernorm(x, axis=-1)
    return x + _A_ref(xn, A_k_cache, A_v_cache, A_wq, A_wo) + _B_ref(xn, B_w_r, B_w_gate, B_w_up, B_w_down)
```

```python
import jax
import jax.numpy as jnp
from jax.experimental import pallas as pl
from jax.experimental.pallas import tpu as pltpu

_HQ = 32
_DH = 128
_EPS = 1e-5
_ROWS = 8


def _build(D, HKV, SK, F, wo_chunks=8):
    HQ, DH = _HQ, _DH
    REP = HQ // HKV
    W = min(4096, max(256, SK // 4))
    RO = (HQ * DH) // wo_chunks
    NSEM = 3 + 2 * HKV + 3 + wo_chunks

    def kernel(x_hbm, k_hbm, v_hbm, wq_hbm, wo_hbm, wr_hbm, wg_hbm, wu_hbm, wd_hbm, o_ref,
               x_v, wr_v, wq_v, k_v, v_v, wg_v, wu_v, wd_v, wo_v, sems):
        pairs = [(x_hbm, x_v), (wr_hbm, wr_v), (wq_hbm, wq_v)]
        for h in range(HKV):
            pairs.append((k_hbm.at[0, h, pl.ds(SK - W, W)], k_v.at[h]))
            pairs.append((v_hbm.at[0, h, pl.ds(SK - W, W)], v_v.at[h]))
        pairs += [(wg_hbm, wg_v), (wu_hbm, wu_v), (wd_hbm, wd_v)]
        for i in range(wo_chunks):
            pairs.append((wo_hbm.at[pl.ds(i * RO, RO)], wo_v.at[pl.ds(i * RO, RO)]))
        copies = [pltpu.make_async_copy(s, d, sems.at[i]) for i, (s, d) in enumerate(pairs)]
        for c in copies:
            c.start()
        c_x, c_wr, c_wq = copies[0:3]
        c_k = copies[3:3 + 2 * HKV:2]
        c_v = copies[4:3 + 2 * HKV:2]
        c_wg, c_wu, c_wd = copies[3 + 2 * HKV:6 + 2 * HKV]
        c_wo = copies[6 + 2 * HKV:]

        c_x.wait()
        x = x_v[0].astype(jnp.float32)
        xc = x - jnp.mean(x, axis=-1, keepdims=True)
        var = jnp.mean(xc * xc, axis=-1, keepdims=True)
        xn = xc * jax.lax.rsqrt(var + _EPS)
        xb = jnp.broadcast_to(xn, (_ROWS, D)).astype(jnp.bfloat16)

        c_wr.wait()
        wr = wr_v[...].reshape(1, D).astype(jnp.float32)
        r = jnp.sum(xb[0:1].astype(jnp.float32) * wr, axis=-1, keepdims=True)
        gate = jax.nn.sigmoid(r)

        c_wq.wait()
        q = jnp.dot(xb, wq_v[...], preferred_element_type=jnp.float32)
        q = q.astype(jnp.bfloat16).astype(jnp.float32)

        row = jax.lax.broadcasted_iota(jnp.int32, (_ROWS, DH), 0)
        row_w = jax.lax.broadcasted_iota(jnp.int32, (_ROWS, REP * DH), 0)
        col_w = jax.lax.broadcasted_iota(jnp.int32, (_ROWS, REP * DH), 1)
        diag = row_w == (col_w // DH)

        o_parts = []
        for h in range(HKV):
            qh = q[:, (REP * h) * DH:(REP * h + 1) * DH]
            for j in range(1, REP):
                qh = jnp.where(row == j, q[:, (REP * h + j) * DH:(REP * h + j + 1) * DH], qh)
            qh = qh.astype(jnp.bfloat16)
            c_k[h].wait()
            s = jax.lax.dot_general(qh, k_v[h], (((1,), (1,)), ((), ())),
                                    preferred_element_type=jnp.float32) * (DH ** -0.5)
            p = jnp.exp(s - jnp.max(s, axis=-1, keepdims=True))
            l = jnp.sum(p, axis=-1, keepdims=True)
            c_v[h].wait()
            o = jnp.dot(p.astype(jnp.bfloat16), v_v[h], preferred_element_type=jnp.float32) / l
            o_parts.append(jnp.where(diag, jnp.concatenate([o] * REP, axis=1), 0.0).astype(jnp.bfloat16))

        c_wg.wait()
        g = jnp.dot(xb, wg_v[...], preferred_element_type=jnp.float32)
        c_wu.wait()
        u = jnp.dot(xb, wu_v[...], preferred_element_type=jnp.float32)
        hh = (g * jax.nn.sigmoid(g) * u).astype(jnp.bfloat16)
        c_wd.wait()
        y = jnp.dot(hh, wd_v[...], preferred_element_type=jnp.float32)

        lo = jnp.concatenate(o_parts, axis=1)
        acc = None
        for i in range(wo_chunks):
            c_wo[i].wait()
            part = jnp.dot(lo[:, i * RO:(i + 1) * RO], wo_v[pl.ds(i * RO, RO), :],
                           preferred_element_type=jnp.float32)
            acc = part if acc is None else acc + part
        attn = jnp.sum(acc, axis=0, keepdims=True)
        out = x + attn + (xn + (xn * 0.0 + y[0:1] * gate))
        o_ref[0] = out.astype(o_ref.dtype)

    return kernel, W, NSEM


@jax.jit
def pallas_parallel_sum__sliding_block_cached__moe_arch_mod__decode_kernel(
    A_x: jax.Array,
    A_k_cache: jax.Array,
    A_v_cache: jax.Array,
    A_wq: jax.Array,
    A_wo: jax.Array,
    B_x: jax.Array,
    B_w_r: jax.Array,
    B_w_gate: jax.Array,
    B_w_up: jax.Array,
    B_w_down: jax.Array,
):
    del B_x
    B, S, D = A_x.shape
    assert (B, S) == (1, 1)
    _, HKV, SK, DH = A_k_cache.shape
    F = B_w_gate.shape[1]
    kernel, W, nsem = _build(D, HKV, SK, F)
    dt = A_x.dtype
    any_spec = pl.BlockSpec(memory_space=pl.ANY)
    return pl.pallas_call(
        kernel,
        out_shape=jax.ShapeDtypeStruct((1, 1, D), dt),
        in_specs=[any_spec] * 9,
        out_specs=pl.BlockSpec(memory_space=pltpu.VMEM),
        scratch_shapes=[
            pltpu.VMEM((1, 1, D), dt),
            pltpu.VMEM((D,), dt),
            pltpu.VMEM((D, _HQ * DH), dt),
            pltpu.VMEM((HKV, W, DH), dt),
            pltpu.VMEM((HKV, W, DH), dt),
            pltpu.VMEM((D, F), dt),
            pltpu.VMEM((D, F), dt),
            pltpu.VMEM((F, D), dt),
            pltpu.VMEM((_HQ * DH, D), dt),
            pltpu.SemaphoreType.DMA((nsem,)),
        ],
        compiler_params=pltpu.CompilerParams(vmem_limit_bytes=64 * 1024 * 1024),
    )(A_x, A_k_cache, A_v_cache, A_wq, A_wo, B_w_r, B_w_gate, B_w_up, B_w_down)
```

```python
import jax
import jax.numpy as jnp
from jax.experimental import pallas as pl
from jax.experimental.pallas import tpu as pltpu

_HQ = 32
_DH = 128
_EPS = 1e-5
_ROWS = 8


def _build(D, HKV, W, SK):
    HQ, DH = _HQ, _DH
    REP = HQ // HKV
    H1 = (5 * HKV) // 8
    HD = HQ * DH
    wo_rows = [r for r in (HD - 768, 640, 128) if r > 0] if HD > 768 else [HD]
    wo_off = [sum(wo_rows[:i]) for i in range(len(wo_rows) + 1)]
    NW = len(wo_rows)
    NG = 2 + NW

    def kernel(x_hbm, k_hbm, v_hbm, wq_hbm, wo_hbm, wr_hbm, wg_hbm, wu_hbm, wd_hbm, o_ref,
               x_v, wr_v, wq_v, k_v, v_v, wg_v, wu_v, wd_v, wo_v, sems):

        def mk(src, dst, g):
            return pltpu.make_async_copy(src, dst, sems.at[g % 2])

        def kv(h0, h1, g):
            out = []
            for h in range(h0, h1):
                out.append(mk(k_hbm.at[0, h, pl.ds(SK - W, W)], k_v.at[h], g))
                out.append(mk(v_hbm.at[0, h, pl.ds(SK - W, W)], v_v.at[h], g))
            return out

        groups = [
            [mk(wq_hbm, wq_v, 0), mk(x_hbm, x_v, 0), mk(wr_hbm, wr_v, 0)] + kv(0, H1, 0),
            kv(H1, HKV, 1) + [mk(wg_hbm, wg_v, 1), mk(wu_hbm, wu_v, 1), mk(wd_hbm, wd_v, 1)],
        ] + [
            [mk(wo_hbm.at[pl.ds(wo_off[i], wo_rows[i])], wo_v.at[pl.ds(wo_off[i], wo_rows[i])], 2 + i)]
            for i in range(NW)
        ]

        def start(g):
            if g < NG:
                for c in groups[g]:
                    c.start()

        def wait(g):
            for c in groups[g]:
                c.wait()
            start(g + 2)

        start(0)
        start(1)

        wait(0)
        x = x_v[0].astype(jnp.float32)
        xc = x - jnp.mean(x, axis=-1, keepdims=True)
        var = jnp.mean(xc * xc, axis=-1, keepdims=True)
        xn = xc * jax.lax.rsqrt(var + _EPS)
        xb = jnp.broadcast_to(xn, (_ROWS, D)).astype(jnp.bfloat16)

        wr = wr_v[...].reshape(1, D).astype(jnp.float32)
        r = jnp.sum(xb[0:1].astype(jnp.float32) * wr, axis=-1, keepdims=True)
        gate = jax.nn.sigmoid(r)

        q = jnp.dot(xb, wq_v[...], preferred_element_type=jnp.float32)
        row = jax.lax.broadcasted_iota(jnp.int32, (_ROWS, DH), 0)

        def head(h):
            qh = q[:, (REP * h) * DH:(REP * h + 1) * DH]
            for j in range(1, REP):
                qh = jnp.where(row == j, q[:, (REP * h + j) * DH:(REP * h + j + 1) * DH], qh)
            s = jax.lax.dot_general(qh.astype(jnp.bfloat16), k_v[h], (((1,), (1,)), ((), ())),
                                    preferred_element_type=jnp.float32) * (DH ** -0.5)
            p = jnp.exp(s - jnp.max(s, axis=-1, keepdims=True))
            l = jnp.sum(p, axis=-1, keepdims=True)
            o = jnp.dot(p.astype(jnp.bfloat16), v_v[h], preferred_element_type=jnp.float32) / l
            return jnp.concatenate(
                [jnp.broadcast_to(o[j:j + 1], (_ROWS, DH)) for j in range(REP)], axis=1
            ).astype(jnp.bfloat16)

        o_parts = [head(h) for h in range(H1)]

        wait(1)
        g = jnp.dot(xb, wg_v[...], preferred_element_type=jnp.float32)
        u = jnp.dot(xb, wu_v[...], preferred_element_type=jnp.float32)
        hh = (g * jax.nn.sigmoid(g) * u).astype(jnp.bfloat16)
        y = jnp.dot(hh, wd_v[...], preferred_element_type=jnp.float32)
        o_parts += [head(h) for h in range(H1, HKV)]

        lo = jnp.concatenate(o_parts, axis=1)
        acc = x + (xn + (xn * 0.0 + y * gate))
        for i in range(NW):
            wait(2 + i)
            acc = acc + jnp.dot(lo[:, wo_off[i]:wo_off[i + 1]], wo_v[pl.ds(wo_off[i], wo_rows[i]), :],
                                preferred_element_type=jnp.float32)
        o_ref[0] = acc[0:1].astype(o_ref.dtype)

    return kernel


@jax.jit
def pallas_parallel_sum__sliding_block_cached__moe_arch_mod__decode_kernel(
    A_x: jax.Array,
    A_k_cache: jax.Array,
    A_v_cache: jax.Array,
    A_wq: jax.Array,
    A_wo: jax.Array,
    B_x: jax.Array,
    B_w_r: jax.Array,
    B_w_gate: jax.Array,
    B_w_up: jax.Array,
    B_w_down: jax.Array,
):
    del B_x
    B, S, D = A_x.shape
    _, HKV, SK, DH = A_k_cache.shape
    assert (B, S, DH) == (1, 1, _DH)
    F = B_w_gate.shape[1]
    W = min(4096, max(256, SK // 4))
    dt = A_x.dtype
    any_spec = pl.BlockSpec(memory_space=pl.ANY)
    return pl.pallas_call(
        _build(D, HKV, W, SK),
        out_shape=jax.ShapeDtypeStruct((1, 1, D), dt),
        in_specs=[any_spec] * 9,
        out_specs=pl.BlockSpec(memory_space=pltpu.VMEM),
        scratch_shapes=[
            pltpu.VMEM((1, 1, D), dt),
            pltpu.VMEM((D,), B_w_r.dtype),
            pltpu.VMEM((D, _HQ * DH), A_wq.dtype),
            pltpu.VMEM((HKV, W, DH), A_k_cache.dtype),
            pltpu.VMEM((HKV, W, DH), A_v_cache.dtype),
            pltpu.VMEM((D, F), B_w_gate.dtype),
            pltpu.VMEM((D, F), B_w_up.dtype),
            pltpu.VMEM((F, D), B_w_down.dtype),
            pltpu.VMEM((_HQ * DH, D), A_wo.dtype),
            pltpu.SemaphoreType.DMA((2,)),
        ],
        compiler_params=pltpu.CompilerParams(vmem_limit_bytes=64 * 1024 * 1024),
    )(A_x, A_k_cache, A_v_cache, A_wq, A_wo, B_w_r, B_w_gate, B_w_up, B_w_down)
```

```python
import jax
import jax.numpy as jnp
from jax.experimental import pallas as pl
from jax.experimental.pallas import tpu as pltpu

_HQ = 32
_DH = 128
_EPS = 1e-5
_ROWS = 8
_NSEM = 3
_MXU_ROWS = (3200, 640)
_VPU_ROWS = (192, 64)


def _build(D, HKV, W, SK):
    HQ, DH = _HQ, _DH
    REP = HQ // HKV
    H1 = (5 * HKV) // 8
    HD = HQ * DH
    wo_rows = _MXU_ROWS + _VPU_ROWS
    wo_off = [sum(wo_rows[:i]) for i in range(len(wo_rows) + 1)]
    assert wo_off[-1] == HD
    NM, NW = len(_MXU_ROWS), len(wo_rows)
    NG = 2 + NW
    VT = pl.cdiv(sum(_VPU_ROWS), 128) * 128

    def kernel(x_hbm, k_hbm, v_hbm, wq_hbm, wo_hbm, wr_hbm, wg_hbm, wu_hbm, wd_hbm, o_ref,
               x_v, wr_v, wq_v, k_v, v_v, wg_v, wu_v, wd_v, wo_v, sems):

        def mk(src, dst, g):
            return pltpu.make_async_copy(src, dst, sems.at[g % _NSEM])

        def kv(h0, h1, g):
            out = []
            for h in range(h0, h1):
                out.append(mk(k_hbm.at[0, h, pl.ds(SK - W, W)], k_v.at[h], g))
                out.append(mk(v_hbm.at[0, h, pl.ds(SK - W, W)], v_v.at[h], g))
            return out

        groups = [
            [mk(wq_hbm, wq_v, 0), mk(x_hbm, x_v, 0), mk(wr_hbm, wr_v, 0)] + kv(0, H1, 0),
            kv(H1, HKV, 1) + [mk(wg_hbm, wg_v, 1), mk(wu_hbm, wu_v, 1), mk(wd_hbm, wd_v, 1)],
        ] + [
            [mk(wo_hbm.at[pl.ds(wo_off[i], wo_rows[i])], wo_v.at[pl.ds(wo_off[i], wo_rows[i])], 2 + i)]
            for i in range(NW)
        ]

        def start(g):
            if g < NG:
                for c in groups[g]:
                    c.start()

        def wait(g):
            for c in groups[g]:
                c.wait()
            start(g + _NSEM)

        for g in range(_NSEM):
            start(g)

        wait(0)
        x = x_v[0].astype(jnp.float32)
        xc = x - jnp.mean(x, axis=-1, keepdims=True)
        var = jnp.mean(xc * xc, axis=-1, keepdims=True)
        xn = xc * jax.lax.rsqrt(var + _EPS)
        xb = jnp.broadcast_to(xn, (_ROWS, D)).astype(jnp.bfloat16)

        wr = wr_v[...].reshape(1, D).astype(jnp.float32)
        r = jnp.sum(xb[0:1].astype(jnp.float32) * wr, axis=-1, keepdims=True)
        gate = jax.nn.sigmoid(r)

        q = jnp.dot(xb, wq_v[...], preferred_element_type=jnp.float32)
        row = jax.lax.broadcasted_iota(jnp.int32, (_ROWS, DH), 0)

        def head(h):
            qh = q[:, (REP * h) * DH:(REP * h + 1) * DH]
            for j in range(1, REP):
                qh = jnp.where(row == j, q[:, (REP * h + j) * DH:(REP * h + j + 1) * DH], qh)
            s = jax.lax.dot_general(qh.astype(jnp.bfloat16), k_v[h], (((1,), (1,)), ((), ())),
                                    preferred_element_type=jnp.float32) * (DH ** -0.5)
            p = jnp.exp(s - jnp.max(s, axis=-1, keepdims=True))
            l = jnp.sum(p, axis=-1, keepdims=True)
            o = jnp.dot(p.astype(jnp.bfloat16), v_v[h], preferred_element_type=jnp.float32) / l
            return jnp.concatenate(
                [jnp.broadcast_to(o[j:j + 1], (_ROWS, DH)) for j in range(REP)], axis=1
            ).astype(jnp.bfloat16)

        o_parts = [head(h) for h in range(H1)]

        wait(1)
        g = jnp.dot(xb, wg_v[...], preferred_element_type=jnp.float32)
        u = jnp.dot(xb, wu_v[...], preferred_element_type=jnp.float32)
        hh = (g * jax.nn.sigmoid(g) * u).astype(jnp.bfloat16)
        y = jnp.dot(hh, wd_v[...], preferred_element_type=jnp.float32)
        o_parts += [head(h) for h in range(H1, HKV)]

        lo = jnp.concatenate(o_parts, axis=1)
        acc = x + (xn + (xn * 0.0 + y * gate))
        ot = jnp.transpose(jnp.broadcast_to(lo[0:1, HD - VT:].astype(jnp.float32), (128, VT)))
        for i in range(NM):
            wait(2 + i)
            acc = acc + jnp.dot(lo[:, wo_off[i]:wo_off[i + 1]], wo_v[pl.ds(wo_off[i], wo_rows[i]), :],
                                preferred_element_type=jnp.float32)
        part = None
        for i in range(NM, NW):
            wait(2 + i)
            n, t0 = wo_rows[i], wo_off[i] - (HD - VT)
            prod = (wo_v[pl.ds(wo_off[i], n), :].astype(jnp.float32)
                    * jnp.concatenate([ot[t0:t0 + n, :]] * (D // 128), axis=1))
            for j in range(n // _ROWS):
                blk = prod[_ROWS * j:_ROWS * (j + 1)]
                part = blk if part is None else part + blk
        out = acc[0:1] + jnp.sum(part, axis=0, keepdims=True)
        o_ref[0] = out.astype(o_ref.dtype)

    return kernel


@jax.jit
def pallas_parallel_sum__sliding_block_cached__moe_arch_mod__decode_kernel(
    A_x: jax.Array,
    A_k_cache: jax.Array,
    A_v_cache: jax.Array,
    A_wq: jax.Array,
    A_wo: jax.Array,
    B_x: jax.Array,
    B_w_r: jax.Array,
    B_w_gate: jax.Array,
    B_w_up: jax.Array,
    B_w_down: jax.Array,
):
    del B_x
    B, S, D = A_x.shape
    _, HKV, SK, DH = A_k_cache.shape
    assert (B, S, DH) == (1, 1, _DH)
    F = B_w_gate.shape[1]
    W = min(4096, max(256, SK // 4))
    dt = A_x.dtype
    any_spec = pl.BlockSpec(memory_space=pl.ANY)
    return pl.pallas_call(
        _build(D, HKV, W, SK),
        out_shape=jax.ShapeDtypeStruct((1, 1, D), dt),
        in_specs=[any_spec] * 9,
        out_specs=pl.BlockSpec(memory_space=pltpu.VMEM),
        scratch_shapes=[
            pltpu.VMEM((1, 1, D), dt),
            pltpu.VMEM((D,), B_w_r.dtype),
            pltpu.VMEM((D, _HQ * DH), A_wq.dtype),
            pltpu.VMEM((HKV, W, DH), A_k_cache.dtype),
            pltpu.VMEM((HKV, W, DH), A_v_cache.dtype),
            pltpu.VMEM((D, F), B_w_gate.dtype),
            pltpu.VMEM((D, F), B_w_up.dtype),
            pltpu.VMEM((F, D), B_w_down.dtype),
            pltpu.VMEM((_HQ * DH, D), A_wo.dtype),
            pltpu.SemaphoreType.DMA((_NSEM,)),
        ],
        compiler_params=pltpu.CompilerParams(vmem_limit_bytes=64 * 1024 * 1024),
    )(A_x, A_k_cache, A_v_cache, A_wq, A_wo, B_w_r, B_w_gate, B_w_up, B_w_down)
```

```python
import jax
import jax.numpy as jnp
from jax.experimental import pallas as pl
from jax.experimental.pallas import tpu as pltpu

_HQ = 32
_DH = 128
_EPS = 1e-5
_ROWS = 8
_NSEM = 3
_MXU_ROWS = (3200, 640)
_VPU_ROWS = (192, 64)


def _build(D, HKV, W, SK):
    HQ, DH = _HQ, _DH
    REP = HQ // HKV
    H1 = (5 * HKV) // 8
    HD = HQ * DH
    wo_rows = _MXU_ROWS + _VPU_ROWS
    wo_off = [sum(wo_rows[:i]) for i in range(len(wo_rows) + 1)]
    assert wo_off[-1] == HD
    NM, NW = len(_MXU_ROWS), len(wo_rows)
    NG = 2 + NW
    VT = pl.cdiv(sum(_VPU_ROWS), 128) * 128

    def compute(x_hbm, k_hbm, v_hbm, wq_hbm, wo_hbm, wr_hbm, wg_hbm, wu_hbm, wd_hbm,
                x_v, wr_v, wq_v, k_v, v_v, wg_v, wu_v, wd_v, wo_v, o_v, sems):

        def mk(src, dst, g):
            return pltpu.make_async_copy(src, dst, sems.at[g % _NSEM])

        def kv(h0, h1, g):
            out = []
            for h in range(h0, h1):
                out.append(mk(k_hbm.at[0, h, pl.ds(SK - W, W)], k_v.at[h], g))
                out.append(mk(v_hbm.at[0, h, pl.ds(SK - W, W)], v_v.at[h], g))
            return out

        groups = [
            [mk(wq_hbm, wq_v, 0), mk(x_hbm, x_v, 0), mk(wr_hbm, wr_v, 0)] + kv(0, H1, 0),
            kv(H1, HKV, 1) + [mk(wg_hbm, wg_v, 1), mk(wu_hbm, wu_v, 1), mk(wd_hbm, wd_v, 1)],
        ] + [
            [mk(wo_hbm.at[pl.ds(wo_off[i], wo_rows[i])], wo_v.at[pl.ds(wo_off[i], wo_rows[i])], 2 + i)]
            for i in range(NW)
        ]

        def start(g):
            if g < NG:
                for c in groups[g]:
                    c.start()

        def wait(g):
            for c in groups[g]:
                c.wait()
            start(g + _NSEM)

        for g in range(_NSEM):
            start(g)

        wait(0)
        x = x_v[0].astype(jnp.float32)
        xc = x - jnp.mean(x, axis=-1, keepdims=True)
        var = jnp.mean(xc * xc, axis=-1, keepdims=True)
        xn = xc * jax.lax.rsqrt(var + _EPS)
        xb = jnp.broadcast_to(xn, (_ROWS, D)).astype(jnp.bfloat16)

        wr = wr_v[...].reshape(1, D).astype(jnp.float32)
        r = jnp.sum(xb[0:1].astype(jnp.float32) * wr, axis=-1, keepdims=True)
        gate = jax.nn.sigmoid(r)

        q = jnp.dot(xb, wq_v[...], preferred_element_type=jnp.float32)
        row = jax.lax.broadcasted_iota(jnp.int32, (_ROWS, DH), 0)

        def head(h):
            qh = q[:, (REP * h) * DH:(REP * h + 1) * DH]
            for j in range(1, REP):
                qh = jnp.where(row == j, q[:, (REP * h + j) * DH:(REP * h + j + 1) * DH], qh)
            s = jax.lax.dot_general(qh.astype(jnp.bfloat16), k_v[h], (((1,), (1,)), ((), ())),
                                    preferred_element_type=jnp.float32) * (DH ** -0.5)
            p = jnp.exp(s - jnp.max(s, axis=-1, keepdims=True))
            l = jnp.sum(p, axis=-1, keepdims=True)
            o = jnp.dot(p.astype(jnp.bfloat16), v_v[h], preferred_element_type=jnp.float32) / l
            return jnp.concatenate(
                [jnp.broadcast_to(o[j:j + 1], (_ROWS, DH)) for j in range(REP)], axis=1
            ).astype(jnp.bfloat16)

        o_parts = [head(h) for h in range(H1)]

        wait(1)
        g = jnp.dot(xb, wg_v[...], preferred_element_type=jnp.float32)
        u = jnp.dot(xb, wu_v[...], preferred_element_type=jnp.float32)
        hh = (g * jax.nn.sigmoid(g) * u).astype(jnp.bfloat16)
        y = jnp.dot(hh, wd_v[...], preferred_element_type=jnp.float32)
        o_parts += [head(h) for h in range(H1, HKV)]

        lo = jnp.concatenate(o_parts, axis=1)
        acc = x + (xn + (xn * 0.0 + y * gate))
        ot = jnp.transpose(jnp.broadcast_to(lo[0:1, HD - VT:].astype(jnp.float32), (128, VT)))
        for i in range(NM):
            wait(2 + i)
            acc = acc + jnp.dot(lo[:, wo_off[i]:wo_off[i + 1]], wo_v[pl.ds(wo_off[i], wo_rows[i]), :],
                                preferred_element_type=jnp.float32)
        part = None
        for i in range(NM, NW):
            wait(2 + i)
            n, t0 = wo_rows[i], wo_off[i] - (HD - VT)
            prod = (wo_v[pl.ds(wo_off[i], n), :].astype(jnp.float32)
                    * jnp.concatenate([ot[t0:t0 + n, :]] * (D // 128), axis=1))
            for j in range(n // _ROWS):
                blk = prod[_ROWS * j:_ROWS * (j + 1)]
                part = blk if part is None else part + blk
        out = acc[0:1] + jnp.sum(part, axis=0, keepdims=True)
        o_v[0] = out.astype(o_v.dtype)

    def kernel(*refs):
        ins, o_hbm, scratch, o_v, o_sem = refs[:9], refs[9], refs[10:19], refs[19], refs[20]
        write_back = pltpu.make_async_copy(o_v, o_hbm, o_sem.at[0])

        def body(sems):
            compute(*ins, *scratch, o_v, sems)
            write_back.start()

        pl.run_scoped(body, pltpu.SemaphoreType.DMA((_NSEM,)))
        write_back.wait()

    return kernel


@jax.jit
def pallas_parallel_sum__sliding_block_cached__moe_arch_mod__decode_kernel(
    A_x: jax.Array,
    A_k_cache: jax.Array,
    A_v_cache: jax.Array,
    A_wq: jax.Array,
    A_wo: jax.Array,
    B_x: jax.Array,
    B_w_r: jax.Array,
    B_w_gate: jax.Array,
    B_w_up: jax.Array,
    B_w_down: jax.Array,
):
    del B_x
    B, S, D = A_x.shape
    _, HKV, SK, DH = A_k_cache.shape
    assert (B, S, DH) == (1, 1, _DH)
    F = B_w_gate.shape[1]
    W = min(4096, max(256, SK // 4))
    dt = A_x.dtype
    any_spec = pl.BlockSpec(memory_space=pl.ANY)
    return pl.pallas_call(
        _build(D, HKV, W, SK),
        out_shape=jax.ShapeDtypeStruct((1, 1, D), dt),
        in_specs=[any_spec] * 9,
        out_specs=any_spec,
        scratch_shapes=[
            pltpu.VMEM((1, 1, D), dt),
            pltpu.VMEM((D,), B_w_r.dtype),
            pltpu.VMEM((D, _HQ * DH), A_wq.dtype),
            pltpu.VMEM((HKV, W, DH), A_k_cache.dtype),
            pltpu.VMEM((HKV, W, DH), A_v_cache.dtype),
            pltpu.VMEM((D, F), B_w_gate.dtype),
            pltpu.VMEM((D, F), B_w_up.dtype),
            pltpu.VMEM((F, D), B_w_down.dtype),
            pltpu.VMEM((_HQ * DH, D), A_wo.dtype),
            pltpu.VMEM((1, 1, D), dt),
            pltpu.SemaphoreType.DMA((1,)),
        ],
        compiler_params=pltpu.CompilerParams(vmem_limit_bytes=64 * 1024 * 1024),
    )(A_x, A_k_cache, A_v_cache, A_wq, A_wo, B_w_r, B_w_gate, B_w_up, B_w_down)
```

```python
import jax
import jax.numpy as jnp
from jax.experimental import pallas as pl
from jax.experimental.pallas import tpu as pltpu

_HQ = 32
_DH = 128
_EPS = 1e-5
_ROWS = 8
_NSEM = 3
_MXU_ROWS = (3200, 640)
_VPU_ROWS = (192, 64)


def _build(D, HKV, W, SK):
    HQ, DH = _HQ, _DH
    REP = HQ // HKV
    H1 = (5 * HKV) // 8
    HD = HQ * DH
    wo_rows = _MXU_ROWS + _VPU_ROWS
    wo_off = [sum(wo_rows[:i]) for i in range(len(wo_rows) + 1)]
    assert wo_off[-1] == HD
    NM, NW = len(_MXU_ROWS), len(wo_rows)
    NG = 2 + NW
    VT = pl.cdiv(sum(_VPU_ROWS), 128) * 128

    def compute(x_hbm, k_hbm, v_hbm, wq_hbm, wo_hbm, wr_hbm, wg_hbm, wu_hbm, wd_hbm,
                x_v, wr_v, wq_v, k0_v, v0_v, k1_v, v1_v, wg_v, wu_v, wd_v, wo_vs, o_v, sems):
        k_v = [k0_v.at[h] for h in range(H1)] + [k1_v.at[h] for h in range(HKV - H1)]
        v_v = [v0_v.at[h] for h in range(H1)] + [v1_v.at[h] for h in range(HKV - H1)]

        def mk(src, dst, g):
            return pltpu.make_async_copy(src, dst, sems.at[g % _NSEM])

        def kv(h0, h1, g):
            out = []
            for h in range(h0, h1):
                out.append(mk(k_hbm.at[0, h, pl.ds(SK - W, W)], k_v[h], g))
                out.append(mk(v_hbm.at[0, h, pl.ds(SK - W, W)], v_v[h], g))
            return out

        groups = [
            [mk(wq_hbm, wq_v, 0), mk(x_hbm, x_v, 0), mk(wr_hbm, wr_v, 0)] + kv(0, H1, 0),
            kv(H1, HKV, 1) + [mk(wg_hbm, wg_v, 1), mk(wu_hbm, wu_v, 1), mk(wd_hbm, wd_v, 1)],
        ] + [
            [mk(wo_hbm.at[pl.ds(wo_off[i], wo_rows[i])], wo_vs[i], 2 + i)] for i in range(NW)
        ]

        def start(g):
            if g < NG:
                for c in groups[g]:
                    c.start()

        def wait(g):
            for c in groups[g]:
                c.wait()
            start(g + _NSEM)

        for g in range(_NSEM):
            start(g)

        wait(0)
        x = x_v[0].astype(jnp.float32)
        xc = x - jnp.mean(x, axis=-1, keepdims=True)
        var = jnp.mean(xc * xc, axis=-1, keepdims=True)
        xn = xc * jax.lax.rsqrt(var + _EPS)
        xb = jnp.broadcast_to(xn, (_ROWS, D)).astype(jnp.bfloat16)

        wr = wr_v[...].reshape(1, D).astype(jnp.float32)
        r = jnp.sum(xb[0:1].astype(jnp.float32) * wr, axis=-1, keepdims=True)
        gate = jax.nn.sigmoid(r)

        q = jnp.dot(xb, wq_v[...], preferred_element_type=jnp.float32)
        row = jax.lax.broadcasted_iota(jnp.int32, (_ROWS, DH), 0)

        def head(h):
            qh = q[:, (REP * h) * DH:(REP * h + 1) * DH]
            for j in range(1, REP):
                qh = jnp.where(row == j, q[:, (REP * h + j) * DH:(REP * h + j + 1) * DH], qh)
            s = jax.lax.dot_general(qh.astype(jnp.bfloat16), k_v[h][...], (((1,), (1,)), ((), ())),
                                    preferred_element_type=jnp.float32) * (DH ** -0.5)
            p = jnp.exp(s - jnp.max(s, axis=-1, keepdims=True))
            l = jnp.sum(p, axis=-1, keepdims=True)
            o = jnp.dot(p.astype(jnp.bfloat16), v_v[h][...], preferred_element_type=jnp.float32) / l
            return jnp.concatenate(
                [jnp.broadcast_to(o[j:j + 1], (_ROWS, DH)) for j in range(REP)], axis=1
            ).astype(jnp.bfloat16)

        o_parts = [head(h) for h in range(H1)]

        wait(1)
        g = jnp.dot(xb, wg_v[...], preferred_element_type=jnp.float32)
        u = jnp.dot(xb, wu_v[...], preferred_element_type=jnp.float32)
        hh = (g * jax.nn.sigmoid(g) * u).astype(jnp.bfloat16)
        y = jnp.dot(hh, wd_v[...], preferred_element_type=jnp.float32)
        o_parts += [head(h) for h in range(H1, HKV)]

        lo = jnp.concatenate(o_parts, axis=1)
        acc = x + (xn + (xn * 0.0 + y * gate))
        ot = jnp.transpose(jnp.broadcast_to(lo[0:1, HD - VT:].astype(jnp.float32), (128, VT)))
        for i in range(NM):
            wait(2 + i)
            acc = acc + jnp.dot(lo[:, wo_off[i]:wo_off[i + 1]], wo_vs[i][...],
                                preferred_element_type=jnp.float32)
        part = None
        for i in range(NM, NW):
            wait(2 + i)
            n, t0 = wo_rows[i], wo_off[i] - (HD - VT)
            prod = (wo_vs[i][...].astype(jnp.float32)
                    * jnp.concatenate([ot[t0:t0 + n, :]] * (D // 128), axis=1))
            for j in range(n // _ROWS):
                blk = prod[_ROWS * j:_ROWS * (j + 1)]
                part = blk if part is None else part + blk
        out = acc[0:1] + jnp.sum(part, axis=0, keepdims=True)
        o_v[0] = out.astype(o_v.dtype)

    def kernel(*refs):
        ins, o_hbm, rest = refs[:9], refs[9], refs[10:]
        bufs, wo_vs, (o_v, o_sem) = rest[:10], rest[10:10 + NW], rest[10 + NW:]
        write_back = pltpu.make_async_copy(o_v, o_hbm, o_sem.at[0])

        def body(sems):
            compute(*ins, *bufs, wo_vs, o_v, sems)
            write_back.start()

        pl.run_scoped(body, pltpu.SemaphoreType.DMA((_NSEM,)))
        write_back.wait()

    return kernel, H1, wo_rows


@jax.jit
def pallas_parallel_sum__sliding_block_cached__moe_arch_mod__decode_kernel(
    A_x: jax.Array,
    A_k_cache: jax.Array,
    A_v_cache: jax.Array,
    A_wq: jax.Array,
    A_wo: jax.Array,
    B_x: jax.Array,
    B_w_r: jax.Array,
    B_w_gate: jax.Array,
    B_w_up: jax.Array,
    B_w_down: jax.Array,
):
    del B_x
    B, S, D = A_x.shape
    _, HKV, SK, DH = A_k_cache.shape
    assert (B, S, DH) == (1, 1, _DH)
    F = B_w_gate.shape[1]
    W = min(4096, max(256, SK // 4))
    dt = A_x.dtype
    any_spec = pl.BlockSpec(memory_space=pl.ANY)
    kernel, H1, wo_rows = _build(D, HKV, W, SK)
    return pl.pallas_call(
        kernel,
        out_shape=jax.ShapeDtypeStruct((1, 1, D), dt),
        in_specs=[any_spec] * 9,
        out_specs=any_spec,
        scratch_shapes=[
            pltpu.VMEM((1, 1, D), dt),
            pltpu.VMEM((D,), B_w_r.dtype),
            pltpu.VMEM((D, _HQ * DH), A_wq.dtype),
            pltpu.VMEM((H1, W, DH), A_k_cache.dtype),
            pltpu.VMEM((H1, W, DH), A_v_cache.dtype),
            pltpu.VMEM((HKV - H1, W, DH), A_k_cache.dtype),
            pltpu.VMEM((HKV - H1, W, DH), A_v_cache.dtype),
            pltpu.VMEM((D, F), B_w_gate.dtype),
            pltpu.VMEM((D, F), B_w_up.dtype),
            pltpu.VMEM((F, D), B_w_down.dtype),
            *[pltpu.VMEM((n, D), A_wo.dtype) for n in wo_rows],
            pltpu.VMEM((1, 1, D), dt),
            pltpu.SemaphoreType.DMA((1,)),
        ],
        compiler_params=pltpu.CompilerParams(vmem_limit_bytes=64 * 1024 * 1024),
    )(A_x, A_k_cache, A_v_cache, A_wq, A_wo, B_w_r, B_w_gate, B_w_up, B_w_down)
```

```python
import jax
import jax.numpy as jnp
from jax.experimental import pallas as pl
from jax.experimental.pallas import tpu as pltpu

_HQ = 32
_DH = 128
_EPS = 1e-5
_ROWS = 8
_MXU_ROWS = (3200, 640)
_VPU_ROWS = (192, 64)


def _build(D, HKV, W, SK):
    HQ, DH = _HQ, _DH
    REP = HQ // HKV
    H1 = (5 * HKV) // 8
    HD = HQ * DH
    wo_rows = _MXU_ROWS + _VPU_ROWS
    wo_off = [sum(wo_rows[:i]) for i in range(len(wo_rows) + 1)]
    assert wo_off[-1] == HD
    NM, NW = len(_MXU_ROWS), len(wo_rows)
    NG = 2 + NW
    VT = pl.cdiv(sum(_VPU_ROWS), 128) * 128

    def compute(x_hbm, k_hbm, v_hbm, wq_hbm, wo_hbm, wr_hbm, wg_hbm, wu_hbm, wd_hbm,
                x_v, wr_v, wq_v, k0_v, v0_v, k1_v, v1_v, wg_v, wu_v, wd_v, wo_vs, o_v, sems):
        k_v = [k0_v.at[h] for h in range(H1)] + [k1_v.at[h] for h in range(HKV - H1)]
        v_v = [v0_v.at[h] for h in range(H1)] + [v1_v.at[h] for h in range(HKV - H1)]

        def mk(src, dst, g):
            return pltpu.make_async_copy(src, dst, sems.at[g])

        def kv(h0, h1, g):
            out = []
            for h in range(h0, h1):
                out.append(mk(k_hbm.at[0, h, pl.ds(SK - W, W)], k_v[h], g))
                out.append(mk(v_hbm.at[0, h, pl.ds(SK - W, W)], v_v[h], g))
            return out

        groups = [
            [mk(wq_hbm, wq_v, 0), mk(x_hbm, x_v, 0), mk(wr_hbm, wr_v, 0)] + kv(0, H1, 0),
            kv(H1, HKV, 1) + [mk(wg_hbm, wg_v, 1), mk(wu_hbm, wu_v, 1), mk(wd_hbm, wd_v, 1)],
        ] + [
            [mk(wo_hbm.at[pl.ds(wo_off[i], wo_rows[i])], wo_vs[i], 2 + i)] for i in range(NW)
        ]

        def wait(g):
            for c in groups[g]:
                c.wait()

        for group in groups:
            for c in group:
                c.start()

        wait(0)
        x = x_v[0].astype(jnp.float32)
        xc = x - jnp.mean(x, axis=-1, keepdims=True)
        var = jnp.mean(xc * xc, axis=-1, keepdims=True)
        xn = xc * jax.lax.rsqrt(var + _EPS)
        xb = jnp.broadcast_to(xn, (_ROWS, D)).astype(jnp.bfloat16)

        wr = wr_v[...].reshape(1, D).astype(jnp.float32)
        r = jnp.sum(xb[0:1].astype(jnp.float32) * wr, axis=-1, keepdims=True)
        gate = jax.nn.sigmoid(r)

        q = jnp.dot(xb, wq_v[...], preferred_element_type=jnp.float32)
        row = jax.lax.broadcasted_iota(jnp.int32, (_ROWS, DH), 0)

        def head(h):
            qh = q[:, (REP * h) * DH:(REP * h + 1) * DH]
            for j in range(1, REP):
                qh = jnp.where(row == j, q[:, (REP * h + j) * DH:(REP * h + j + 1) * DH], qh)
            s = jax.lax.dot_general(qh.astype(jnp.bfloat16), k_v[h][...], (((1,), (1,)), ((), ())),
                                    preferred_element_type=jnp.float32) * (DH ** -0.5)
            p = jnp.exp(s - jnp.max(s, axis=-1, keepdims=True))
            l = jnp.sum(p, axis=-1, keepdims=True)
            o = jnp.dot(p.astype(jnp.bfloat16), v_v[h][...], preferred_element_type=jnp.float32) / l
            return jnp.concatenate(
                [jnp.broadcast_to(o[j:j + 1], (_ROWS, DH)) for j in range(REP)], axis=1
            ).astype(jnp.bfloat16)

        o_parts = [head(h) for h in range(H1)]

        wait(1)
        g = jnp.dot(xb, wg_v[...], preferred_element_type=jnp.float32)
        u = jnp.dot(xb, wu_v[...], preferred_element_type=jnp.float32)
        hh = (g * jax.nn.sigmoid(g) * u).astype(jnp.bfloat16)
        y = jnp.dot(hh, wd_v[...], preferred_element_type=jnp.float32)
        o_parts += [head(h) for h in range(H1, HKV)]

        lo = jnp.concatenate(o_parts, axis=1)
        acc = x + (xn + (xn * 0.0 + y * gate))
        ot = jnp.transpose(jnp.broadcast_to(lo[0:1, HD - VT:].astype(jnp.float32), (128, VT)))
        for i in range(NM):
            wait(2 + i)
            acc = acc + jnp.dot(lo[:, wo_off[i]:wo_off[i + 1]], wo_vs[i][...],
                                preferred_element_type=jnp.float32)
        part = None
        for i in range(NM, NW):
            wait(2 + i)
            n, t0 = wo_rows[i], wo_off[i] - (HD - VT)
            prod = (wo_vs[i][...].astype(jnp.float32)
                    * jnp.concatenate([ot[t0:t0 + n, :]] * (D // 128), axis=1))
            for j in range(n // _ROWS):
                blk = prod[_ROWS * j:_ROWS * (j + 1)]
                part = blk if part is None else part + blk
        out = acc[0:1] + jnp.sum(part, axis=0, keepdims=True)
        o_v[0] = out.astype(o_v.dtype)

    def kernel(*refs):
        ins, o_hbm, rest = refs[:9], refs[9], refs[10:]
        bufs, wo_vs, (o_v, o_sem) = rest[:10], rest[10:10 + NW], rest[10 + NW:]
        write_back = pltpu.make_async_copy(o_v, o_hbm, o_sem.at[0])

        def body(sems):
            compute(*ins, *bufs, wo_vs, o_v, sems)
            write_back.start()

        pl.run_scoped(body, pltpu.SemaphoreType.DMA((NG,)))
        write_back.wait()

    return kernel, H1, wo_rows


@jax.jit
def pallas_parallel_sum__sliding_block_cached__moe_arch_mod__decode_kernel(
    A_x: jax.Array,
    A_k_cache: jax.Array,
    A_v_cache: jax.Array,
    A_wq: jax.Array,
    A_wo: jax.Array,
    B_x: jax.Array,
    B_w_r: jax.Array,
    B_w_gate: jax.Array,
    B_w_up: jax.Array,
    B_w_down: jax.Array,
):
    del B_x
    B, S, D = A_x.shape
    _, HKV, SK, DH = A_k_cache.shape
    assert (B, S, DH) == (1, 1, _DH)
    F = B_w_gate.shape[1]
    W = min(4096, max(256, SK // 4))
    dt = A_x.dtype
    any_spec = pl.BlockSpec(memory_space=pl.ANY)
    kernel, H1, wo_rows = _build(D, HKV, W, SK)
    return pl.pallas_call(
        kernel,
        out_shape=jax.ShapeDtypeStruct((1, 1, D), dt),
        in_specs=[any_spec] * 9,
        out_specs=any_spec,
        scratch_shapes=[
            pltpu.VMEM((1, 1, D), dt),
            pltpu.VMEM((D,), B_w_r.dtype),
            pltpu.VMEM((D, _HQ * DH), A_wq.dtype),
            pltpu.VMEM((H1, W, DH), A_k_cache.dtype),
            pltpu.VMEM((H1, W, DH), A_v_cache.dtype),
            pltpu.VMEM((HKV - H1, W, DH), A_k_cache.dtype),
            pltpu.VMEM((HKV - H1, W, DH), A_v_cache.dtype),
            pltpu.VMEM((D, F), B_w_gate.dtype),
            pltpu.VMEM((D, F), B_w_up.dtype),
            pltpu.VMEM((F, D), B_w_down.dtype),
            *[pltpu.VMEM((n, D), A_wo.dtype) for n in wo_rows],
            pltpu.VMEM((1, 1, D), dt),
            pltpu.SemaphoreType.DMA((1,)),
        ],
        compiler_params=pltpu.CompilerParams(vmem_limit_bytes=64 * 1024 * 1024),
    )(A_x, A_k_cache, A_v_cache, A_wq, A_wo, B_w_r, B_w_gate, B_w_up, B_w_down)
```
